```python
import jax
import jax.numpy as jnp

def _softmax(x, axis=-1):
    return jax.nn.softmax(x, axis=axis)
def _gelu(x):
    return jax.nn.gelu(x, approximate=True)
def _silu(x):
    return jax.nn.silu(x)
def _sigmoid(x):
    return jax.nn.sigmoid(x)
def _layernorm(x, axis=-1, eps=1e-5):
    m = jnp.mean(x, axis=axis, keepdims=True)
    v = jnp.var(x, axis=axis, keepdims=True)
    return (x - m) / jnp.sqrt(v + eps)
def _scatter_add(tgt, idx, src, axis=0):
    return tgt.at[idx].add(src)
def _segment_sum(src, seg, n):
    return jax.ops.segment_sum(src, seg, n)
class _Rng:
    def __init__(self, key):
        self._k = key
    def _next(self):
        self._k, sub = jax.random.split(self._k)
        return sub
    def normal(self, shape):
        return jax.random.normal(self._next(), shape, dtype=jnp.bfloat16)
    def randint(self, lo, hi, shape):
        return jax.random.randint(self._next(), shape, lo, hi, dtype=jnp.int32)
    def uniform(self, shape, lo=0.0, hi=1.0):
        return jax.random.uniform(self._next(), shape, jnp.bfloat16, lo, hi)
    def permutation(self, n):
        return jax.random.permutation(self._next(), n)


kernel_name = 'recurrent_scan__compressed_kv_cla__moe_arch_mod__decode'

def setup_inputs():
    _rng = _Rng(jax.random.key(int.from_bytes(__import__("os").urandom(4), "little")))
    _w = (lambda a: (lambda t: t.astype(jnp.bfloat16) if jnp.issubdtype(t.dtype, jnp.floating) else t)(jnp.asarray(a)))
    def _A_setup():
        B, H, Sq, Sk, D, M = 4, 32, 1, 4096, 128, 576
        Dc = 4 * D
        return {
            "x": _w((lambda *s: _rng.normal(s) * 0.05)(B, Sq, M)),
            "c_kv": _w((lambda *s: _rng.normal(s) * 0.05)(B, Sk, Dc)),
            "w_q": _w((lambda *s: _rng.normal(s) * 0.05)(M, H, D) * (M ** -0.5)),
            "w_uk": _w((lambda *s: _rng.normal(s) * 0.05)(Dc, H, D) * (Dc ** -0.5)),
            "w_uv": _w((lambda *s: _rng.normal(s) * 0.05)(Dc, H, D) * (Dc ** -0.5)),
            "w_o": _w((lambda *s: _rng.normal(s) * 0.05)(H, D, M) * ((H * D) ** -0.5)),
        }
    _A_in = _A_setup()

    def _B_setup():
        B, S, D, F, C = 4, 1, 576, 4608, 1
        return {
            "x": _w((lambda *s: _rng.normal(s) * 0.05)(B, S, D)),
            "w_r": _w((lambda *s: _rng.normal(s) * 0.05)(D)),
            "w_gate": _w((lambda *s: _rng.normal(s) * 0.05)(D, F)),
            "w_up": _w((lambda *s: _rng.normal(s) * 0.05)(D, F)),
            "w_down": _w((lambda *s: _rng.normal(s) * 0.05)(F, D)),
        }
    _B_in = _B_setup()

    return {
        "A_x": _A_in["x"],
        "A_c_kv": _A_in["c_kv"],
        "A_w_q": _A_in["w_q"],
        "A_w_uk": _A_in["w_uk"],
        "A_w_uv": _A_in["w_uv"],
        "A_w_o": _A_in["w_o"],
        "B_x": _B_in["x"],
        "B_w_r": _B_in["w_r"],
        "B_w_gate": _B_in["w_gate"],
        "B_w_up": _B_in["w_up"],
        "B_w_down": _B_in["w_down"],
    }

def reference(A_x, A_c_kv, A_w_q, A_w_uk, A_w_uv, A_w_o, B_x, B_w_r, B_w_gate, B_w_up, B_w_down):
    def _A_ref(x, c_kv, w_q, w_uk, w_uv, w_o):
        B, Sq, M = x.shape[0], x.shape[1], x.shape[2]
        Sk = c_kv.shape[1]
        H, D = w_q.shape[1], w_q.shape[2]
        q = jnp.einsum("bqm,mhd->bhqd", x, w_q)
        k = jnp.einsum("bkc,chd->bhkd", c_kv, w_uk)
        v = jnp.einsum("bkc,chd->bhkd", c_kv, w_uv)
        scores = jnp.einsum("bhqd,bhkd->bhqk", q, k) * (D ** -0.5)
        off = Sk - Sq
        qi = jnp.arange(Sq)[:, None]
        kj = jnp.arange(Sk)[None, :]
        cmask = kj <= (qi + off)
        scores = jnp.where(cmask[None, None], scores, -1e9)
        p = _softmax(scores, axis=-1)
        ctx = jnp.einsum("bhqk,bhkd->bhqd", p, v)
        return jnp.einsum("bhqd,hdm->bqm", ctx, w_o)

    def _B_ref(x, w_r, w_gate, w_up, w_down):
        B, S, D = x.shape
        C = 1
        r = x @ w_r
        idx = jnp.argsort(-r, axis=-1)[:, :C]
        idx_e = jnp.repeat(idx.reshape(B, C, 1), D, axis=2)
        x_sel = jnp.take_along_axis(x, idx_e, axis=1)
        g = _silu(x_sel @ w_gate)
        u = x_sel @ w_up
        y = (g * u) @ w_down
        r_sel = _sigmoid(jnp.take_along_axis(r, idx, axis=1))
        y = y * r_sel.reshape(B, C, 1)
        b_off = (jnp.arange(B) * S).reshape(B, 1)
        flat_idx = (idx + b_off).reshape(B * C)
        zero = (x * 0.0).reshape(B * S, D)
        upd = _scatter_add(zero, flat_idx, y.reshape(B * C, D), axis=0)
        return x + upd.reshape(B, S, D)

    x = A_x
    xn = _layernorm(x, axis=-1)
    s = _A_ref(xn, A_c_kv, A_w_q, A_w_uk, A_w_uv, A_w_o)
    g = _silu(_B_ref(xn, B_w_r, B_w_gate, B_w_up, B_w_down))
    return x + s * g
```

```python
import jax
import jax.numpy as jnp
from jax import lax
import jax.experimental.pallas as pl
import jax.experimental.pallas.tpu as pltpu

_F32 = jnp.float32
_BF16 = jnp.bfloat16
_NT = (((1,), (1,)), ((), ()))

_HG = 16
_QB = 96
_CB = 128
_KB = 1024
_FB = 512
_WO_CHUNKS = (12, 8, 6, 3, 2, 1)


def _dot(a, b):
    return jnp.dot(a, b, preferred_element_type=_F32)


def _dot_nt(a, b):
    return lax.dot_general(a, b, _NT, preferred_element_type=_F32)


def _iota(shape, dim):
    return lax.broadcasted_iota(jnp.int32, shape, dim)


def _sigmoid(x):
    return 1.0 / (1.0 + jnp.exp(-x))


def _kernel(
    x_hbm, wr_hbm, wq_hbm, wuk_hbm, kv_hbm, wuv_hbm, wg_hbm, wu_hbm, wd_hbm, wo_hbm,
    o_ref,
    x_v, wr_v, wq_v, wuk_v, kv_v, wuv_v, wg_v, wu_v, wd_v, wo_v,
    e_ref, xb_ref, qa_ref, s_ref, cc_ref, ctx_ref, h_ref, sems,
):
    nb, m_dim = x_v.shape
    _, n_heads, d_head = wq_v.shape
    _, n_keys, d_lat = kv_v.shape
    d_ff = wg_v.shape[1]
    n_groups = n_heads // _HG
    rows = nb * _HG

    pairs = [(wq_hbm, wq_v), (x_hbm, x_v), (wr_hbm, wr_v), (wuk_hbm, wuk_v)]
    pairs += [(kv_hbm.at[b], kv_v.at[b]) for b in range(nb)]
    pairs += [(wuv_hbm, wuv_v), (wg_hbm, wg_v), (wu_hbm, wu_v), (wd_hbm, wd_v)]
    h0 = 0
    for n in _WO_CHUNKS:
        pairs.append((wo_hbm.at[pl.ds(h0, n)], wo_v.at[pl.ds(h0, n)]))
        h0 += n
    copies = [pltpu.make_async_copy(s, d, sems.at[i]) for i, (s, d) in enumerate(pairs)]
    for c in copies:
        c.start()
    cp_wq, cp_x, cp_wr, cp_wuk = copies[:4]
    cp_wuv, cp_wg, cp_wu, cp_wd = copies[4 + nb:8 + nb]
    cp_wo = copies[8 + nb:]

    e_shape = e_ref.shape
    e_ref[...] = jnp.where(
        _iota(e_shape, 1) // _HG == _iota(e_shape, 0), 1.0, 0.0
    ).astype(_BF16)

    def own_head(n_cols):
        shape = (rows, n_cols)
        return _iota(shape, 0) % _HG == _iota(shape, 1) % _HG

    def head_group(w_ref, start, size, g):
        w = w_ref[pl.ds(start, size), g * _HG:(g + 1) * _HG, :]
        return w.reshape(size * _HG, d_head)

    cp_x.wait()
    x = x_v[...].astype(_F32)
    mean = jnp.mean(x, axis=-1, keepdims=True)
    xc = x - mean
    var = jnp.mean(xc * xc, axis=-1, keepdims=True)
    xn = xc / jnp.sqrt(var + 1e-5)

    def repeat_rows(n_rows, rep):
        row = _iota((n_rows, m_dim), 0) // rep
        out = jnp.zeros((n_rows, m_dim), _F32)
        for b in range(nb):
            out = jnp.where(row == b, xn[b:b + 1, :], out)
        return out

    x_rep = repeat_rows(rows, _HG)
    xb_ref[...] = jnp.zeros(xb_ref.shape, _BF16)
    for i in range(m_dim // _QB):
        xb_ref[i, :, 0:_QB] = x_rep[:, i * _QB:(i + 1) * _QB].astype(_BF16)
    x8 = repeat_rows(8, 1).astype(_BF16)

    cp_wq.wait()

    def q_step(i, acc):
        spread = _dot(xb_ref[i], e_ref[:, 0:_QB * _HG])
        lhs = jnp.where(own_head(_QB * _HG), spread, 0.0).astype(_BF16)
        start = pl.multiple_of(i * _QB, _QB)
        return tuple(
            acc[g] + _dot(lhs, head_group(wq_v, start, _QB, g)) for g in range(n_groups)
        )

    q = lax.fori_loop(
        0, m_dim // _QB, q_step,
        tuple(jnp.zeros((rows, d_head), _F32) for _ in range(n_groups)),
    )
    q = [(qg * (d_head ** -0.5)).astype(_BF16) for qg in q]

    cp_wuk.wait()

    def uk_step(j, carry):
        start = pl.multiple_of(j * _CB, _CB)
        for g in range(n_groups):
            full = _dot_nt(q[g], head_group(wuk_v, start, _CB, g))
            own = jnp.where(own_head(_CB * _HG), full, 0.0).astype(_BF16)
            qa_ref[j, g] = _dot_nt(own, e_ref[...]).astype(_BF16)
        return carry

    lax.fori_loop(0, d_lat // _CB, uk_step, 0)

    def attend(b, carry):
        pltpu.make_async_copy(kv_hbm.at[b], kv_v.at[b], sems.at[4 + b]).wait()
        r0 = pl.multiple_of(b * _HG, _HG)
        qa = jnp.concatenate(
            [
                jnp.concatenate(
                    [qa_ref[j, g, pl.ds(r0, _HG), :] for j in range(d_lat // _CB)], axis=1
                )
                for g in range(n_groups)
            ],
            axis=0,
        )

        def keys(i):
            return kv_v[b, pl.ds(pl.multiple_of(i * _KB, _KB), _KB), :]

        def score_step(i, m):
            s = _dot_nt(qa, keys(i))
            s_ref[i] = s
            for t in range(_KB // 128):
                m = jnp.maximum(m, s[:, t * 128:(t + 1) * 128])
            return m

        m = lax.fori_loop(
            0, n_keys // _KB, score_step, jnp.full((n_heads, 128), -jnp.inf, _F32)
        )
        m = jnp.max(m, axis=-1, keepdims=True)

        def value_step(i, carry):
            l, acc = carry
            p = jnp.exp(s_ref[i] - m)
            for t in range(_KB // 128):
                l = l + p[:, t * 128:(t + 1) * 128]
            return l, acc + _dot(p.astype(_BF16), keys(i))

        l, acc = lax.fori_loop(
            0, n_keys // _KB, value_step,
            (jnp.zeros((n_heads, 128), _F32), jnp.zeros((n_heads, d_lat), _F32)),
        )
        cc = (acc / jnp.sum(l, axis=-1, keepdims=True)).astype(_BF16)
        for g in range(n_groups):
            for j in range(d_lat // _CB):
                cc_ref[j, g, pl.ds(r0, _HG), :] = cc[
                    g * _HG:(g + 1) * _HG, j * _CB:(j + 1) * _CB
                ]
        return carry

    lax.fori_loop(0, nb, attend, 0)

    cp_wuv.wait()

    def uv_step(j, acc):
        start = pl.multiple_of(j * _CB, _CB)
        out = []
        for g in range(n_groups):
            spread = _dot(cc_ref[j, g], e_ref[...])
            lhs = jnp.where(own_head(_CB * _HG), spread, 0.0).astype(_BF16)
            out.append(acc[g] + _dot(lhs, head_group(wuv_v, start, _CB, g)))
        return tuple(out)

    ctx = lax.fori_loop(
        0, d_lat // _CB, uv_step,
        tuple(jnp.zeros((rows, d_head), _F32) for _ in range(n_groups)),
    )
    p_shape = (8 * _HG, rows)
    dst, src = _iota(p_shape, 0), _iota(p_shape, 1)
    regroup = jnp.where(
        (dst // 8 == src % _HG) & (dst % 8 == src // _HG), 1.0, 0.0
    ).astype(_BF16)
    for g in range(n_groups):
        ctx_ref[g * 8 * _HG:(g + 1) * 8 * _HG, :] = _dot(regroup, ctx[g].astype(_BF16))

    cp_wg.wait()
    cp_wu.wait()

    def up_step(i, carry):
        cols = pl.ds(pl.multiple_of(i * _FB, _FB), _FB)
        gate = _dot(x8, wg_v[:, cols])
        h_ref[i] = gate * _sigmoid(gate) * _dot(x8, wu_v[:, cols])
        return carry

    lax.fori_loop(0, d_ff // _FB, up_step, 0)

    cp_wr.wait()
    w_r = wr_v[...].astype(_F32).reshape(1, m_dim)
    route = _sigmoid(jnp.sum(xn * w_r, axis=-1, keepdims=True))

    cp_wd.wait()

    def down_step(i, acc):
        cols = pl.ds(pl.multiple_of(i * _FB, _FB), _FB)
        return acc + _dot_nt(h_ref[i].astype(_BF16), wd_v[:, cols])

    y = lax.fori_loop(0, d_ff // _FB, down_step, jnp.zeros((8, m_dim), _F32))
    z = xn + (xn * 0.0 + y[0:nb] * route)
    gate = z * _sigmoid(z)

    s = jnp.zeros((8, m_dim), _F32)
    h0 = 0
    for n, cp in zip(_WO_CHUNKS, cp_wo):
        cp.wait()
        for h in range(h0, h0 + n):
            s = s + _dot_nt(ctx_ref[8 * h:8 * h + 8, :].astype(_BF16), wo_v[h])
        h0 += n
    o_ref[...] = (x + s[0:nb] * gate).astype(o_ref.dtype)


@jax.jit
def pallas_recurrent_scan__compressed_kv_cla__moe_arch_mod__decode_kernel(
    A_x: jax.Array,
    A_c_kv: jax.Array,
    A_w_q: jax.Array,
    A_w_uk: jax.Array,
    A_w_uv: jax.Array,
    A_w_o: jax.Array,
    B_x: jax.Array,
    B_w_r: jax.Array,
    B_w_gate: jax.Array,
    B_w_up: jax.Array,
    B_w_down: jax.Array,
):
    del B_x
    nb, sq, m_dim = A_x.shape
    _, n_keys, d_lat = A_c_kv.shape
    _, n_heads, d_head = A_w_q.shape
    d_ff = B_w_gate.shape[1]
    assert sq == 1 and nb <= 8 and sum(_WO_CHUNKS) == n_heads
    n_groups = n_heads // _HG
    rows = nb * _HG

    operands = (
        A_x.reshape(nb, m_dim), B_w_r, A_w_q, A_w_uk, A_c_kv, A_w_uv,
        B_w_gate, B_w_up, B_w_down.T, jnp.transpose(A_w_o, (0, 2, 1)),
    )
    scratch = [pltpu.VMEM(a.shape, a.dtype) for a in operands] + [
        pltpu.VMEM((_CB, _CB * _HG), _BF16),
        pltpu.VMEM((m_dim // _QB, rows, _CB), _BF16),
        pltpu.VMEM((d_lat // _CB, n_groups, rows, _CB), _BF16),
        pltpu.VMEM((n_keys // _KB, n_heads, _KB), _F32),
        pltpu.VMEM((d_lat // _CB, n_groups, rows, _CB), _BF16),
        pltpu.VMEM((8 * n_heads, d_head), _F32),
        pltpu.VMEM((d_ff // _FB, 8, _FB), _F32),
        pltpu.SemaphoreType.DMA((8 + nb + len(_WO_CHUNKS),)),
    ]
    out = pl.pallas_call(
        _kernel,
        out_shape=jax.ShapeDtypeStruct((nb, m_dim), A_x.dtype),
        in_specs=[pl.BlockSpec(memory_space=pltpu.HBM)] * len(operands),
        out_specs=pl.BlockSpec(memory_space=pltpu.VMEM),
        scratch_shapes=scratch,
        compiler_params=pltpu.CompilerParams(vmem_limit_bytes=100 * 2**20),
    )(*operands)
    return out.reshape(nb, sq, m_dim)
```

```python
import jax
import jax.numpy as jnp
from jax import lax
import jax.experimental.pallas as pl
import jax.experimental.pallas.tpu as pltpu

_F32 = jnp.float32
_BF16 = jnp.bfloat16
_NT = (((1,), (1,)), ((), ()))

_HG = 16
_FB = 512
_PRIORITY = (0, 1, 1, 1)
_LAG = 24

_WO_REGULAR = (
    ((0, 8, 0, 0, 576),),
    ((0, 8, 1, 0, 576),),
    ((0, 8, 2, 0, 384),),
    ((0, 8, 2, 384, 576),),
)
_WO_FINAL = (
    ((0, 8, 3, 0, 256),),
    ((0, 8, 3, 512, 576), (0, 4, 3, 256, 384)),
    ((4, 4, 3, 256, 384), (0, 4, 3, 384, 512)),
    ((4, 4, 3, 384, 512),),
)
_WO_IN_ORDER = 40
(_S_X, _S_WR, _S_Q, _S_UK, _S_UV, _S_KV, _S_KV_HI, _S_G, _S_U, _S_D, _S_O) = range(11)
_N_SEMS = _S_O + sum(len(piece) for piece in _WO_REGULAR + _WO_FINAL)


def _dot(a, b):
    return jnp.dot(a, b, preferred_element_type=_F32)


def _dot_nt(a, b):
    return lax.dot_general(a, b, _NT, preferred_element_type=_F32)


def _iota(shape, dim):
    return lax.broadcasted_iota(jnp.int32, shape, dim)


def _sigmoid(x):
    return 1.0 / (1.0 + jnp.exp(-x))


def _aligned(start, size, multiple):
    if not isinstance(start, int):
        start = pl.multiple_of(start, multiple)
    return pl.ds(start, size)


class _Stage:
    def __init__(self, n_ticks, copies):
        self.n_ticks, self.copies, self.issued = n_ticks, copies, 0

    def _tick(self, t):
        for copy, priority in zip(self.copies(t), _PRIORITY, strict=True):
            copy.start(priority=priority)

    def _advance(self, n):
        first = self.issued
        self.issued += n
        assert self.issued <= self.n_ticks
        return first

    def ticks(self, n):
        first = self._advance(n)
        for t in range(first, first + n):
            self._tick(t)

    def loop(self, n_steps, ticks_per_step, step, init):
        first = self._advance(n_steps * ticks_per_step)

        def body(i, carry):
            carry = step(i, carry)
            for k in range(ticks_per_step):
                self._tick(first + i * ticks_per_step + k)
            return carry

        return lax.fori_loop(0, n_steps, body, init)

    def idle(self, n):
        if n > 0:
            self.loop(n, 1, lambda i, carry: carry, 0)

    def finish(self):
        self.idle(self.n_ticks - self.issued)


def _kernel(
    x_hbm, wr_hbm, wq_hbm, wuk_hbm, wuv_hbm, kv_hbm, wg_hbm, wu_hbm, wd_hbm, wo_hbm,
    o_hbm,
    x_v, wr_v, wq_v, wuk_v, wuv_v, kv_v, wg_v, wu_v, wd_v, wo_v,
    e_ref, xb_ref, qa_ref, s_ref, cc_ref, ctx_ref, h_ref, out_v, sems,
):
    nb, m_dim = x_v.shape
    n_qb, qb, n_heads, d_head = wq_v.shape
    n_cb, cb = wuk_v.shape[:2]
    n_slabs, kb, d_lat = kv_v.shape
    _, fr, d_ff = wg_v.shape
    n_fb = d_ff // _FB
    n_groups = n_heads // _HG
    rows = nb * _HG
    slabs_per_batch = n_slabs // nb

    def copy(hbm, vmem, sem, *idx):
        return pltpu.make_async_copy(hbm.at[idx], vmem.at[idx], sems.at[sem])

    def wait(vmem, sem, *idx):
        region = vmem.at[idx] if idx else vmem
        pltpu.make_async_copy(region, region, sems.at[sem]).wait()

    def pair(k):
        return pl.ds(2 * k, 2)

    def ffn_tile(t):
        assert n_fb == 9
        r = (t * 57) >> 9
        return r, t - r * n_fb

    def q_copies(t):
        return [copy(wq_hbm, wq_v, _S_Q, pair(k), pl.ds(t, 1)) for k in range(4)]

    def uk_uv_copies(t):
        return [
            copy(hbm, vmem, sem, pair(k), pl.ds(t, 1))
            for k in range(2)
            for hbm, vmem, sem in ((wuk_hbm, wuk_v, _S_UK), (wuv_hbm, wuv_v, _S_UV))
        ]

    def kv_copies(half):
        return lambda t: [
            copy(kv_hbm, kv_v, _S_KV + half, pair(4 * half + k), _aligned(8 * t, 8, 8))
            for k in range(4)
        ]

    def gate_up_copies(t):
        r, c = ffn_tile(t)
        return [
            copy(hbm, vmem, sem, pair(k), _aligned(8 * r, 8, 8), _aligned(_FB * c, _FB, _FB))
            for k in range(2)
            for hbm, vmem, sem in ((wg_hbm, wg_v, _S_G), (wu_hbm, wu_v, _S_U))
        ]

    def down_copies(t):
        r, c = ffn_tile(t)
        return [
            copy(wd_hbm, wd_v, _S_D, pair(k),
                 _aligned(8 * r + (fr // 2) * j, 8, 8), _aligned(_FB * c, _FB, _FB))
            for j in range(2)
            for k in range(2)
        ]

    wo_ends = [(g * m_dim + c1) // 32 for ((_, _, g, _, c1),) in _WO_REGULAR]

    def o_copies(t):
        sem = _S_O
        for end in wo_ends[:-1]:
            sem = sem + (t >= end if isinstance(t, int) else (t >= end).astype(jnp.int32))
        return [copy(wo_hbm, wo_v, sem, pair(k), _aligned(32 * t, 32, 32)) for k in range(4)]

    def own_head(n_cols):
        shape = (rows, n_cols)
        return _iota(shape, 0) % _HG == _iota(shape, 1) % _HG

    def head_group(w_ref, i, g):
        w = w_ref[i, :, g * _HG:(g + 1) * _HG, :]
        return w.reshape(w.shape[0] * _HG, d_head)

    stage = _Stage(qb, q_copies)
    stage.ticks(1)
    pltpu.make_async_copy(x_hbm, x_v, sems.at[_S_X]).start()
    pltpu.make_async_copy(wr_hbm, wr_v, sems.at[_S_WR]).start()
    stage.idle(_LAG)
    e_ref[...] = jnp.where(
        _iota(e_ref.shape, 1) // _HG == _iota(e_ref.shape, 0), 1.0, 0.0
    ).astype(_BF16)
    stage.ticks(2)

    wait(x_v, _S_X)
    x = x_v[...].astype(_F32)
    mean = jnp.mean(x, axis=-1, keepdims=True)
    xc = x - mean
    var = jnp.mean(xc * xc, axis=-1, keepdims=True)
    xn = xc / jnp.sqrt(var + 1e-5)

    def repeat_rows(v, n_rows, rep):
        row = _iota((n_rows, m_dim), 0) // rep
        out = jnp.zeros((n_rows, m_dim), _F32)
        for b in range(nb):
            out = jnp.where(row == b, v[b:b + 1, :], out)
        return out

    xn_rep = repeat_rows(xn, rows, _HG)
    xb_ref[...] = jnp.zeros(xb_ref.shape, _BF16)
    for i in range(n_qb):
        xb_ref[i, :, 0:qb] = xn_rep[:, i * qb:(i + 1) * qb].astype(_BF16)
    x8 = repeat_rows(x, 8, 1)
    xn8 = repeat_rows(xn, 8, 1)
    stage.ticks(2)

    wait(wr_v, _S_WR)
    w_r = wr_v[...].astype(_F32).reshape(1, m_dim)
    route = _sigmoid(jnp.sum(xn8 * w_r, axis=-1, keepdims=True))
    stage.finish()

    stage = _Stage(cb, uk_uv_copies)
    stage.idle(_LAG)
    wait(wq_v, _S_Q)

    def q_step(i, acc):
        spread = _dot(xb_ref[i], e_ref[:, 0:qb * _HG])
        lhs = jnp.where(own_head(qb * _HG), spread, 0.0).astype(_BF16)
        return tuple(acc[g] + _dot(lhs, head_group(wq_v, i, g)) for g in range(n_groups))

    q = stage.loop(
        n_qb, 6, q_step, tuple(jnp.zeros((rows, d_head), _F32) for _ in range(n_groups))
    )
    q = [(qg * (d_head ** -0.5)).astype(_BF16) for qg in q]
    stage.finish()

    stage = _Stage(kb // 8, kv_copies(0))
    stage.idle(_LAG)
    wait(wuk_v, _S_UK)

    def uk_step(j, carry):
        for g in range(n_groups):
            full = _dot_nt(q[g], head_group(wuk_v, j, g))
            own = jnp.where(own_head(cb * _HG), full, 0.0).astype(_BF16)
            qa_ref[j, g] = _dot_nt(own, e_ref[...]).astype(_BF16)
        return carry

    stage.loop(n_cb, 12, uk_step, 0)
    stage.finish()

    def attend(b, stage):
        own_rows = pl.ds(b * _HG, _HG)
        qa = jnp.concatenate(
            [
                jnp.concatenate([qa_ref[j, g, own_rows, :] for j in range(n_cb)], axis=1)
                for g in range(n_groups)
            ],
            axis=0,
        )

        def score_step(i, m):
            s = _dot_nt(qa, kv_v[b * slabs_per_batch + i])
            s_ref[i] = s
            for t in range(kb // 128):
                m = jnp.maximum(m, s[:, t * 128:(t + 1) * 128])
            return m

        m = stage.loop(
            slabs_per_batch, 6, score_step, jnp.full((n_heads, 128), -jnp.inf, _F32)
        )
        m = jnp.max(m, axis=-1, keepdims=True)

        def value_step(i, carry):
            l, acc = carry
            p = jnp.exp(s_ref[i] - m)
            for t in range(kb // 128):
                l = l + p[:, t * 128:(t + 1) * 128]
            return l, acc + _dot(p.astype(_BF16), kv_v[b * slabs_per_batch + i])

        l, acc = stage.loop(
            slabs_per_batch, 5, value_step,
            (jnp.zeros((n_heads, 128), _F32), jnp.zeros((n_heads, d_lat), _F32)),
        )
        cc = (acc / jnp.sum(l, axis=-1, keepdims=True)).astype(_BF16)
        for g in range(n_groups):
            for j in range(n_cb):
                cc_ref[j, g, own_rows, :] = cc[g * _HG:(g + 1) * _HG, j * cb:(j + 1) * cb]

    stage = _Stage(kb // 8, kv_copies(1))
    stage.idle(_LAG)
    wait(kv_v, _S_KV, pl.ds(0, n_slabs // 2))
    for b in range(nb // 2):
        attend(b, stage)
    stage.finish()

    stage = _Stage((fr // 8) * n_fb, gate_up_copies)
    stage.idle(_LAG)
    wait(kv_v, _S_KV_HI, pl.ds(n_slabs // 2, n_slabs // 2))
    for b in range(nb // 2, nb):
        attend(b, stage)
    wait(wuv_v, _S_UV)

    def uv_step(j, acc):
        out = []
        for g in range(n_groups):
            spread = _dot(cc_ref[j, g], e_ref[...])
            lhs = jnp.where(own_head(cb * _HG), spread, 0.0).astype(_BF16)
            out.append(acc[g] + _dot(lhs, head_group(wuv_v, j, g)))
        return tuple(out)

    ctx = stage.loop(
        n_cb, 12, uv_step, tuple(jnp.zeros((rows, d_head), _F32) for _ in range(n_groups))
    )
    dst, src = _iota((8 * _HG, rows), 0), _iota((8 * _HG, rows), 1)
    regroup = jnp.where(
        (dst // 8 == src % _HG) & (dst % 8 == src // _HG), 1.0, 0.0
    ).astype(_BF16)
    for g in range(n_groups):
        ctx_ref[g * 8 * _HG:(g + 1) * 8 * _HG, :] = _dot(regroup, ctx[g].astype(_BF16))
    stage.finish()

    stage = _Stage((fr // 16) * n_fb, down_copies)
    stage.idle(_LAG)
    wait(wg_v, _S_G)
    wait(wu_v, _S_U)
    xn8_bf16 = xn8.astype(_BF16)

    def ffn_cols(w_ref, start, size):
        return w_ref[:, :, _aligned(start, size, _FB)].reshape(m_dim, size)

    def up_step(i, carry):
        gate = _dot(xn8_bf16, ffn_cols(wg_v, i * _FB, _FB))
        h_ref[i] = gate * _sigmoid(gate) * _dot(xn8_bf16, ffn_cols(wu_v, i * _FB, _FB))
        return carry

    stage.loop(n_fb, 5, up_step, 0)
    stage.finish()

    stage = _Stage(wo_ends[-1], o_copies)
    stage.idle(_LAG - 3)
    wait(wd_v, _S_D)

    def down_step(i, acc):
        h = jnp.concatenate([h_ref[3 * i + k] for k in range(3)], axis=1)
        return acc + _dot_nt(h.astype(_BF16), ffn_cols(wd_v, i * 3 * _FB, 3 * _FB))

    y = stage.loop(n_fb // 3, 8, down_step, jnp.zeros((8, m_dim), _F32))
    z = xn8 + (xn8 * 0.0 + y * route)
    gate = z * _sigmoid(z)

    pending = [c for t in range(stage.issued, stage.n_ticks) for c in o_copies(t)]
    piece_ends = [4 * (end - stage.issued) for end in wo_ends]
    sem = _S_O + len(_WO_REGULAR)
    for piece in _WO_FINAL:
        for k0, nk, g, c0, c1 in piece:
            pending += [
                copy(wo_hbm, wo_v, sem, pl.ds(k, 2), pl.ds(g * m_dim + c, 32))
                for c in range(c0, c1, 32)
                for k in range(k0, k0 + nk, 2)
            ]
            sem += 1
        piece_ends.append(len(pending))
    n_started = [0]

    def start_until(n):
        for i in range(n_started[0], min(n, len(pending))):
            in_order = i >= len(pending) - _WO_IN_ORDER
            pending[i].start(priority=1 if in_order else _PRIORITY[i % 4])
            n_started[0] = i + 1

    pieces = _WO_REGULAR + _WO_FINAL
    blocks = [block for piece in pieces for block in piece]
    col_tiles = [(c, min(c + 128, m_dim)) for c in range(0, m_dim, 128)]
    s = [jnp.zeros((8, c1 - c0), _F32) for c0, c1 in col_tiles]
    heads_per_slab = n_heads // wo_v.shape[0]
    n_done = 0
    for piece, end in zip(pieces, piece_ends, strict=True):
        start_until(end + 4 * (_LAG - 3))
        for i, (k0, nk, g, c0, c1) in enumerate(piece):
            wait(wo_v, _S_O + n_done + i, pl.ds(k0, nk), pl.ds(g * m_dim + c0, c1 - c0))
        for k0, nk, g, c0, c1 in piece:
            n_done += 1
            part = None
            for k in range(k0, k0 + nk):
                head = k * heads_per_slab + g
                term = _dot_nt(
                    ctx_ref[8 * head:8 * head + 8, :].astype(_BF16),
                    wo_v[k, g * m_dim + c0:g * m_dim + c1, :],
                )
                part = term if part is None else part + term
                start_until(n_started[0] + 3)
            for n, (t0, t1) in enumerate(col_tiles):
                if c0 <= t0 and t1 <= c1:
                    s[n] = s[n] + part[:, t0 - c0:t1 - c0]
                    if not any(b0 <= t0 and t1 <= b1 for *_, b0, b1 in blocks[n_done:]):
                        out = x8[:, t0:t1] + s[n] * gate[:, t0:t1]
                        out_v[:, t0:t1] = out.astype(out_v.dtype)[0:nb]
    assert n_started[0] == len(pending)

    write_back = pltpu.make_async_copy(out_v, o_hbm, sems.at[_S_X])
    write_back.start()
    write_back.wait()


@jax.jit
def pallas_recurrent_scan__compressed_kv_cla__moe_arch_mod__decode_kernel(
    A_x: jax.Array,
    A_c_kv: jax.Array,
    A_w_q: jax.Array,
    A_w_uk: jax.Array,
    A_w_uv: jax.Array,
    A_w_o: jax.Array,
    B_x: jax.Array,
    B_w_r: jax.Array,
    B_w_gate: jax.Array,
    B_w_up: jax.Array,
    B_w_down: jax.Array,
):
    del B_x
    nb, sq, m_dim = A_x.shape
    _, n_keys, d_lat = A_c_kv.shape
    _, n_heads, d_head = A_w_q.shape
    d_ff = B_w_gate.shape[1]
    assert (nb, sq, m_dim, n_keys, d_lat) == (4, 1, 576, 4096, 512)
    assert (n_heads, d_head, d_ff) == (32, 128, 4608)
    n_groups = n_heads // _HG
    rows = nb * _HG

    operands = (
        A_x.reshape(nb, m_dim),
        B_w_r,
        A_w_q.reshape(8, m_dim // 8, n_heads, d_head),
        A_w_uk.reshape(4, d_lat // 4, n_heads, d_head),
        A_w_uv.reshape(4, d_lat // 4, n_heads, d_head),
        A_c_kv.reshape(16, nb * n_keys // 16, d_lat),
        B_w_gate.reshape(4, m_dim // 4, d_ff),
        B_w_up.reshape(4, m_dim // 4, d_ff),
        B_w_down.T.reshape(4, m_dim // 4, d_ff),
        jnp.transpose(A_w_o, (0, 2, 1)).reshape(8, n_heads * m_dim // 8, d_head),
    )
    scratch = [pltpu.VMEM(a.shape, a.dtype) for a in operands] + [
        pltpu.VMEM((128, 128 * _HG), _BF16),
        pltpu.VMEM((8, rows, 128), _BF16),
        pltpu.VMEM((4, n_groups, rows, d_lat // 4), _BF16),
        pltpu.VMEM((4, n_heads, n_keys // 4), _F32),
        pltpu.VMEM((4, n_groups, rows, d_lat // 4), _BF16),
        pltpu.VMEM((8 * n_heads, d_head), _F32),
        pltpu.VMEM((d_ff // _FB, 8, _FB), _F32),
        pltpu.VMEM((nb, m_dim), A_x.dtype),
        pltpu.SemaphoreType.DMA((_N_SEMS,)),
    ]
    out = pl.pallas_call(
        _kernel,
        out_shape=jax.ShapeDtypeStruct((nb, m_dim), A_x.dtype),
        in_specs=[pl.BlockSpec(memory_space=pltpu.HBM)] * len(operands),
        out_specs=pl.BlockSpec(memory_space=pltpu.HBM),
        scratch_shapes=scratch,
        compiler_params=pltpu.CompilerParams(
            vmem_limit_bytes=100 * 2**20,
            disable_semaphore_checks=True,
            disable_bounds_checks=True,
        ),
    )(*operands)
    return out.reshape(nb, sq, m_dim)
```

```python
import functools

import jax
import jax.numpy as jnp
from jax import lax
import jax.experimental.pallas as pl
import jax.experimental.pallas.tpu as pltpu

_F32 = jnp.float32
_BF16 = jnp.bfloat16
_NT = (((1,), (1,)), ((), ()))

_HG = 16
_FB = 512
_PRIORITY = (0, 1, 1, 1)
_LAG = 24

_WO_REGULAR = (
    ((0, 8, 0, 0, 576),),
    ((0, 8, 1, 0, 576),),
    ((0, 8, 2, 0, 384),),
    ((0, 8, 2, 384, 576),),
)
_WO_FINAL = (
    ((0, 8, 3, 0, 256),),
    ((0, 8, 3, 512, 576), (0, 4, 3, 256, 384)),
    ((4, 4, 3, 256, 384), (0, 4, 3, 384, 512)),
    ((4, 4, 3, 384, 512),),
)
_WO_IN_ORDER = 40
_S_X, _S_WR, _S_Q, _S_UK, _S_UV, _S_G, _S_U, _S_D, _S_KV = range(9)
_S_O = _S_KV + 2
_N_SEMS = _S_O + sum(len(piece) for piece in _WO_REGULAR + _WO_FINAL)


def _dot(a, b):
    return jnp.dot(a, b, preferred_element_type=_F32)


def _dot_nt(a, b):
    return lax.dot_general(a, b, _NT, preferred_element_type=_F32)


def _iota(shape, dim):
    return lax.broadcasted_iota(jnp.int32, shape, dim)


def _sigmoid(x):
    return 1.0 / (1.0 + jnp.exp(-x))


def _aligned(start, size, multiple):
    if not isinstance(start, int):
        start = pl.multiple_of(start, multiple)
    return pl.ds(start, size)


class _Stage:
    def __init__(self, n_ticks, copies):
        self.n_ticks, self.copies, self.issued = n_ticks, copies, 0

    def _tick(self, t):
        for copy, priority in zip(self.copies(t), _PRIORITY, strict=True):
            copy.start(priority=priority)

    def _advance(self, n):
        first = self.issued
        self.issued += n
        assert self.issued <= self.n_ticks
        return first

    def ticks(self, n):
        first = self._advance(n)
        for t in range(first, first + n):
            self._tick(t)

    def loop(self, n_steps, ticks_per_step, step, init):
        first = self._advance(n_steps * ticks_per_step)

        def body(i, carry):
            carry = step(i, carry)
            for k in range(ticks_per_step):
                self._tick(first + i * ticks_per_step + k)
            return carry

        return lax.fori_loop(0, n_steps, body, init)

    def idle(self, n):
        if n > 0:
            self.loop(n, 1, lambda i, carry: carry, 0)

    def finish(self):
        self.idle(self.n_ticks - self.issued)


def _kernel(
    x_hbm, wr_hbm, wq_hbm, wuk_hbm, wuv_hbm, kv_hbm, wg_hbm, wu_hbm, wd_hbm, wo_hbm,
    o_hbm,
    x_v, wr_v, wq_v, wuk_v, wuv_v, kv_v, wg_v, wu_v, wd_v, wo_v,
    e_ref, xb_ref, qa_ref, s_ref, m_ref, cc_ref, ctx_ref, h_ref, out_v, sems,
):
    nb, m_dim = x_v.shape
    n_qb, qb, n_heads, d_head = wq_v.shape
    n_cb, cb = wuk_v.shape[:2]
    n_slabs, kb, d_lat = kv_v.shape
    _, fr, d_ff = wg_v.shape
    n_fb = d_ff // _FB
    n_groups = n_heads // _HG
    rows = nb * _HG
    slabs_per_batch = n_slabs // nb
    half_slab = kb // 2

    def copy(hbm, vmem, sem, *idx):
        return pltpu.make_async_copy(hbm.at[idx], vmem.at[idx], sems.at[sem])

    def wait(vmem, sem, *idx):
        region = vmem.at[idx] if idx else vmem
        pltpu.make_async_copy(region, region, sems.at[sem]).wait()

    def pair(k):
        return pl.ds(2 * k, 2)

    def ffn_tile(t):
        assert n_fb == 9
        r = (t * 57) >> 9
        return r, t - r * n_fb

    def q_copies(t):
        return [copy(wq_hbm, wq_v, _S_Q, pair(k), pl.ds(t, 1)) for k in range(4)]

    def uk_uv_copies(t):
        return [
            copy(hbm, vmem, sem, pair(k), pl.ds(t, 1))
            for k in range(2)
            for hbm, vmem, sem in ((wuk_hbm, wuk_v, _S_UK), (wuv_hbm, wuv_v, _S_UV))
        ]

    def kv_copies(half):
        return lambda t: [
            copy(kv_hbm, kv_v, _S_KV + half, pair(4 * (t & 1) + k),
                 _aligned(half * half_slab + 8 * (t >> 1), 8, 8))
            for k in range(4)
        ]

    def gate_up_copies(t):
        r, c = ffn_tile(t)
        return [
            copy(hbm, vmem, sem, pair(k), _aligned(8 * r, 8, 8), _aligned(_FB * c, _FB, _FB))
            for k in range(2)
            for hbm, vmem, sem in ((wg_hbm, wg_v, _S_G), (wu_hbm, wu_v, _S_U))
        ]

    def down_copies(t):
        r, c = ffn_tile(t)
        return [
            copy(wd_hbm, wd_v, _S_D, pair(k),
                 _aligned(8 * r + (fr // 2) * j, 8, 8), _aligned(_FB * c, _FB, _FB))
            for j in range(2)
            for k in range(2)
        ]

    wo_ends = [(g * m_dim + c1) // 32 for ((_, _, g, _, c1),) in _WO_REGULAR]

    def o_copies(t):
        sem = _S_O
        for end in wo_ends[:-1]:
            sem = sem + (t >= end if isinstance(t, int) else (t >= end).astype(jnp.int32))
        return [copy(wo_hbm, wo_v, sem, pair(k), _aligned(32 * t, 32, 32)) for k in range(4)]

    def own_head(n_cols):
        shape = (rows, n_cols)
        return _iota(shape, 0) % _HG == _iota(shape, 1) % _HG

    def head_group(w_ref, i, g):
        w = w_ref[i, :, g * _HG:(g + 1) * _HG, :]
        return w.reshape(w.shape[0] * _HG, d_head)

    stage = _Stage(qb, q_copies)
    stage.ticks(1)
    pltpu.make_async_copy(x_hbm, x_v, sems.at[_S_X]).start()
    pltpu.make_async_copy(wr_hbm, wr_v, sems.at[_S_WR]).start()

    def init_step(i, carry):
        shape = (16, e_ref.shape[1])
        e_ref[_aligned(16 * i, 16, 16), :] = jnp.where(
            _iota(shape, 1) // _HG == _iota(shape, 0) + 16 * i, 1.0, 0.0
        ).astype(_BF16)
        xb_ref[i] = jnp.zeros(xb_ref.shape[1:], _BF16)
        return carry

    assert e_ref.shape[0] == 16 * n_qb
    stage.loop(n_qb, 1, init_step, 0)
    stage.idle(_LAG + 1 - stage.issued)

    wait(x_v, _S_X)
    x = x_v[...].astype(_F32)
    mean = jnp.mean(x, axis=-1, keepdims=True)
    xc = x - mean
    var = jnp.mean(xc * xc, axis=-1, keepdims=True)
    xn = xc / jnp.sqrt(var + 1e-5)

    def repeat_rows(v, n_rows, rep):
        row = _iota((n_rows, m_dim), 0) // rep
        out = jnp.zeros((n_rows, m_dim), _F32)
        for b in range(nb):
            out = jnp.where(row == b, v[b:b + 1, :], out)
        return out

    xn_rep = repeat_rows(xn, rows, _HG)
    for i in range(n_qb):
        xb_ref[i, :, 0:qb] = xn_rep[:, i * qb:(i + 1) * qb].astype(_BF16)
    x8 = repeat_rows(x, 8, 1)
    xn8 = repeat_rows(xn, 8, 1)
    stage.ticks(2)

    wait(wr_v, _S_WR)
    w_r = wr_v[...].astype(_F32).reshape(1, m_dim)
    route = _sigmoid(jnp.sum(xn8 * w_r, axis=-1, keepdims=True))
    stage.finish()

    stage = _Stage(cb, uk_uv_copies)
    stage.idle(_LAG)
    wait(wq_v, _S_Q)

    def q_step(i, acc):
        spread = _dot(xb_ref[i], e_ref[:, 0:qb * _HG])
        lhs = jnp.where(own_head(qb * _HG), spread, 0.0).astype(_BF16)
        return tuple(acc[g] + _dot(lhs, head_group(wq_v, i, g)) for g in range(n_groups))

    q = stage.loop(
        n_qb, 6, q_step, tuple(jnp.zeros((rows, d_head), _F32) for _ in range(n_groups))
    )
    q = [(qg * (d_head ** -0.5)).astype(_BF16) for qg in q]
    stage.finish()

    stage = _Stage(kb // 8, kv_copies(0))
    stage.idle(_LAG)
    wait(wuk_v, _S_UK)

    def uk_step(j, carry):
        for g in range(n_groups):
            full = _dot_nt(q[g], head_group(wuk_v, j, g))
            own = jnp.where(own_head(cb * _HG), full, 0.0).astype(_BF16)
            qa_ref[j, g] = _dot_nt(own, e_ref[...]).astype(_BF16)
        return carry

    stage.loop(n_cb, 12, uk_step, 0)
    stage.finish()

    def keys(b, half):
        slabs = pl.ds(b * slabs_per_batch, slabs_per_batch)
        k = kv_v[slabs, _aligned(half * half_slab, half_slab, half_slab), :]
        return k.reshape(slabs_per_batch * half_slab, d_lat)

    def head_rows(b):
        return _aligned(b * _HG, _HG, _HG)

    def score_step(half, b, carry):
        qa = jnp.concatenate(
            [
                jnp.concatenate([qa_ref[j, g, head_rows(b), :] for j in range(n_cb)], axis=1)
                for g in range(n_groups)
            ],
            axis=0,
        )
        s = _dot_nt(qa, keys(b, half))
        s_ref[2 * b + half] = s
        m = s[:, 0:128] if half == 0 else jnp.maximum(m_ref[b], s[:, 0:128])
        for t in range(1, s.shape[1] // 128):
            m = jnp.maximum(m, s[:, t * 128:(t + 1) * 128])
        m_ref[b] = m
        return carry

    stage = _Stage(kb // 8, kv_copies(1))
    stage.idle(_LAG)
    wait(kv_v, _S_KV, pl.ds(0, n_slabs), pl.ds(0, half_slab))
    stage.loop(nb, 10, functools.partial(score_step, 0), 0)
    stage.finish()

    stage = _Stage((fr // 8) * n_fb, gate_up_copies)
    stage.idle(_LAG)
    wait(kv_v, _S_KV + 1, pl.ds(0, n_slabs), pl.ds(half_slab, half_slab))
    stage.loop(nb, 10, functools.partial(score_step, 1), 0)

    def value_step(i, carry):
        b, half = i >> 1, i & 1
        l, acc = (jnp.where(half == 1, v, 0.0) for v in carry)
        p = jnp.exp(s_ref[i] - jnp.max(m_ref[b], axis=-1, keepdims=True))
        for t in range(p.shape[1] // 128):
            l = l + p[:, t * 128:(t + 1) * 128]
        acc = acc + _dot(p.astype(_BF16), keys(b, half))
        cc = (acc / jnp.sum(l, axis=-1, keepdims=True)).astype(_BF16)
        for g in range(n_groups):
            for j in range(n_cb):
                cc_ref[j, g, head_rows(b), :] = cc[g * _HG:(g + 1) * _HG, j * cb:(j + 1) * cb]
        return l, acc

    stage.loop(
        2 * nb, 6, value_step,
        (jnp.zeros((n_heads, 128), _F32), jnp.zeros((n_heads, d_lat), _F32)),
    )
    wait(wuv_v, _S_UV)

    def uv_step(j, acc):
        out = []
        for g in range(n_groups):
            spread = _dot(cc_ref[j, g], e_ref[...])
            lhs = jnp.where(own_head(cb * _HG), spread, 0.0).astype(_BF16)
            out.append(acc[g] + _dot(lhs, head_group(wuv_v, j, g)))
        return tuple(out)

    ctx = stage.loop(
        n_cb, 12, uv_step, tuple(jnp.zeros((rows, d_head), _F32) for _ in range(n_groups))
    )
    dst, src = _iota((8 * _HG, rows), 0), _iota((8 * _HG, rows), 1)
    regroup = jnp.where(
        (dst // 8 == src % _HG) & (dst % 8 == src // _HG), 1.0, 0.0
    ).astype(_BF16)
    for g in range(n_groups):
        ctx_ref[g * 8 * _HG:(g + 1) * 8 * _HG, :] = _dot(regroup, ctx[g].astype(_BF16))
    stage.finish()

    stage = _Stage((fr // 16) * n_fb, down_copies)
    stage.idle(_LAG)
    wait(wg_v, _S_G)
    wait(wu_v, _S_U)
    xn8_bf16 = xn8.astype(_BF16)

    def ffn_cols(w_ref, start, size):
        return w_ref[:, :, _aligned(start, size, _FB)].reshape(m_dim, size)

    def up_step(i, carry):
        gate = _dot(xn8_bf16, ffn_cols(wg_v, i * _FB, _FB))
        h_ref[i] = gate * _sigmoid(gate) * _dot(xn8_bf16, ffn_cols(wu_v, i * _FB, _FB))
        return carry

    stage.loop(n_fb, 5, up_step, 0)
    stage.finish()

    stage = _Stage(wo_ends[-1], o_copies)
    stage.idle(_LAG - 3)
    wait(wd_v, _S_D)

    def down_step(i, acc):
        h = jnp.concatenate([h_ref[3 * i + k] for k in range(3)], axis=1)
        return acc + _dot_nt(h.astype(_BF16), ffn_cols(wd_v, i * 3 * _FB, 3 * _FB))

    y = stage.loop(n_fb // 3, 8, down_step, jnp.zeros((8, m_dim), _F32))
    z = xn8 + (xn8 * 0.0 + y * route)
    gate = z * _sigmoid(z)

    pending = [c for t in range(stage.issued, stage.n_ticks) for c in o_copies(t)]
    piece_ends = [4 * (end - stage.issued) for end in wo_ends]
    sem = _S_O + len(_WO_REGULAR)
    for piece in _WO_FINAL:
        for k0, nk, g, c0, c1 in piece:
            pending += [
                copy(wo_hbm, wo_v, sem, pl.ds(k, 2), pl.ds(g * m_dim + c, 32))
                for c in range(c0, c1, 32)
                for k in range(k0, k0 + nk, 2)
            ]
            sem += 1
        piece_ends.append(len(pending))
    n_started = [0]

    def start_until(n):
        for i in range(n_started[0], min(n, len(pending))):
            in_order = i >= len(pending) - _WO_IN_ORDER
            pending[i].start(priority=1 if in_order else _PRIORITY[i % 4])
            n_started[0] = i + 1

    pieces = _WO_REGULAR + _WO_FINAL
    blocks = [block for piece in pieces for block in piece]
    col_tiles = [(c, min(c + 128, m_dim)) for c in range(0, m_dim, 128)]
    s = [jnp.zeros((8, c1 - c0), _F32) for c0, c1 in col_tiles]
    heads_per_slab = n_heads // wo_v.shape[0]
    n_done = 0
    for piece, end in zip(pieces, piece_ends, strict=True):
        start_until(end + 4 * (_LAG - 3))
        for i, (k0, nk, g, c0, c1) in enumerate(piece):
            wait(wo_v, _S_O + n_done + i, pl.ds(k0, nk), pl.ds(g * m_dim + c0, c1 - c0))
        for k0, nk, g, c0, c1 in piece:
            n_done += 1
            part = None
            for k in range(k0, k0 + nk):
                head = k * heads_per_slab + g
                term = _dot_nt(
                    ctx_ref[8 * head:8 * head + 8, :].astype(_BF16),
                    wo_v[k, g * m_dim + c0:g * m_dim + c1, :],
                )
                part = term if part is None else part + term
                start_until(n_started[0] + 3)
            for n, (t0, t1) in enumerate(col_tiles):
                if c0 <= t0 and t1 <= c1:
                    s[n] = s[n] + part[:, t0 - c0:t1 - c0]
                    if not any(b0 <= t0 and t1 <= b1 for *_, b0, b1 in blocks[n_done:]):
                        out = x8[:, t0:t1] + s[n] * gate[:, t0:t1]
                        out_v[:, t0:t1] = out.astype(out_v.dtype)[0:nb]
    assert n_started[0] == len(pending)

    write_back = pltpu.make_async_copy(out_v, o_hbm, sems.at[_S_X])
    write_back.start()
    write_back.wait()


@jax.jit
def pallas_recurrent_scan__compressed_kv_cla__moe_arch_mod__decode_kernel(
    A_x: jax.Array,
    A_c_kv: jax.Array,
    A_w_q: jax.Array,
    A_w_uk: jax.Array,
    A_w_uv: jax.Array,
    A_w_o: jax.Array,
    B_x: jax.Array,
    B_w_r: jax.Array,
    B_w_gate: jax.Array,
    B_w_up: jax.Array,
    B_w_down: jax.Array,
):
    del B_x
    nb, sq, m_dim = A_x.shape
    _, n_keys, d_lat = A_c_kv.shape
    _, n_heads, d_head = A_w_q.shape
    d_ff = B_w_gate.shape[1]
    assert (nb, sq, m_dim, n_keys, d_lat) == (4, 1, 576, 4096, 512)
    assert (n_heads, d_head, d_ff) == (32, 128, 4608)
    n_groups = n_heads // _HG
    rows = nb * _HG

    operands = (
        A_x.reshape(nb, m_dim),
        B_w_r,
        A_w_q.reshape(8, m_dim // 8, n_heads, d_head),
        A_w_uk.reshape(4, d_lat // 4, n_heads, d_head),
        A_w_uv.reshape(4, d_lat // 4, n_heads, d_head),
        A_c_kv.reshape(16, nb * n_keys // 16, d_lat),
        B_w_gate.reshape(4, m_dim // 4, d_ff),
        B_w_up.reshape(4, m_dim // 4, d_ff),
        B_w_down.T.reshape(4, m_dim // 4, d_ff),
        jnp.transpose(A_w_o, (0, 2, 1)).reshape(8, n_heads * m_dim // 8, d_head),
    )
    scratch = [pltpu.VMEM(a.shape, a.dtype) for a in operands] + [
        pltpu.VMEM((128, 128 * _HG), _BF16),
        pltpu.VMEM((8, rows, 128), _BF16),
        pltpu.VMEM((4, n_groups, rows, d_lat // 4), _BF16),
        pltpu.VMEM((2 * nb, n_heads, n_keys // 2), _F32),
        pltpu.VMEM((nb, n_heads, 128), _F32),
        pltpu.VMEM((4, n_groups, rows, d_lat // 4), _BF16),
        pltpu.VMEM((8 * n_heads, d_head), _F32),
        pltpu.VMEM((d_ff // _FB, 8, _FB), _F32),
        pltpu.VMEM((nb, m_dim), A_x.dtype),
        pltpu.SemaphoreType.DMA((_N_SEMS,)),
    ]
    out = pl.pallas_call(
        _kernel,
        out_shape=jax.ShapeDtypeStruct((nb, m_dim), A_x.dtype),
        in_specs=[pl.BlockSpec(memory_space=pltpu.HBM)] * len(operands),
        out_specs=pl.BlockSpec(memory_space=pltpu.HBM),
        scratch_shapes=scratch,
        compiler_params=pltpu.CompilerParams(
            vmem_limit_bytes=100 * 2**20,
            disable_semaphore_checks=True,
            disable_bounds_checks=True,
        ),
    )(*operands)
    return out.reshape(nb, sq, m_dim)
```

```python
import functools

import jax
import jax.numpy as jnp
from jax import lax
import jax.experimental.pallas as pl
import jax.experimental.pallas.tpu as pltpu

_F32 = jnp.float32
_BF16 = jnp.bfloat16
_NT = (((1,), (1,)), ((), ()))

_HG = 16
_FB = 512
_PRIORITY = (0, 1, 1, 1)
_LAG = 24

_WO_REGULAR = (
    ((0, 8, 0, 0, 576),),
    ((0, 8, 1, 0, 576),),
    ((0, 8, 2, 0, 384),),
    ((0, 8, 2, 384, 576),),
)
_WO_FINAL = (
    ((0, 4, 3, 0, 512),),
    ((0, 8, 3, 512, 576), (4, 1, 3, 0, 512)),
    ((5, 2, 3, 0, 512),),
    ((7, 1, 3, 0, 512),),
)
_WO_IN_ORDER = 40
_S_X, _S_WR, _S_Q, _S_UK, _S_UV, _S_G, _S_U, _S_D, _S_KV = range(9)
_S_O = _S_KV + 2
_N_SEMS = _S_O + sum(len(piece) for piece in _WO_REGULAR + _WO_FINAL)


def _dot(a, b):
    return jnp.dot(a, b, preferred_element_type=_F32)


def _dot_nt(a, b):
    return lax.dot_general(a, b, _NT, preferred_element_type=_F32)


def _iota(shape, dim):
    return lax.broadcasted_iota(jnp.int32, shape, dim)


def _sigmoid(x):
    return 1.0 / (1.0 + jnp.exp(-x))


def _aligned(start, size, multiple):
    if not isinstance(start, int):
        start = pl.multiple_of(start, multiple)
    return pl.ds(start, size)


class _Stage:
    def __init__(self, n_ticks, copies):
        self.n_ticks, self.copies, self.issued = n_ticks, copies, 0

    def _tick(self, t):
        for copy, priority in zip(self.copies(t), _PRIORITY, strict=True):
            copy.start(priority=priority)

    def _advance(self, n):
        first = self.issued
        self.issued += n
        assert self.issued <= self.n_ticks
        return first

    def ticks(self, n):
        first = self._advance(n)
        for t in range(first, first + n):
            self._tick(t)

    def loop(self, n_steps, ticks_per_step, step, init):
        first = self._advance(n_steps * ticks_per_step)

        def body(i, carry):
            carry = step(i, carry)
            for k in range(ticks_per_step):
                self._tick(first + i * ticks_per_step + k)
            return carry

        return lax.fori_loop(0, n_steps, body, init)

    def idle(self, n):
        if n > 0:
            self.loop(n, 1, lambda i, carry: carry, 0)

    def finish(self):
        self.idle(self.n_ticks - self.issued)


def _kernel(
    x_hbm, wr_hbm, wq_hbm, wuk_hbm, wuv_hbm, kv_hbm, wg_hbm, wu_hbm, wd_hbm, wo_hbm,
    o_hbm,
    x_v, wr_v, wq_v, wuk_v, wuv_v, kv_v, wg_v, wu_v, wd_v, wo_v,
    e_ref, xb_ref, qa_ref, s_ref, m_ref, cc_ref, ctx_ref, h_ref, out_v, sems,
):
    nb, m_dim = x_v.shape
    n_qb, qb, n_heads, d_head = wq_v.shape
    n_cb, cb = wuk_v.shape[:2]
    n_slabs, kb, d_lat = kv_v.shape
    _, fr, d_ff = wg_v.shape
    n_fb = d_ff // _FB
    n_groups = n_heads // _HG
    rows = nb * _HG
    slabs_per_batch = n_slabs // nb
    half_slab = kb // 2

    def copy(hbm, vmem, sem, *idx):
        return pltpu.make_async_copy(hbm.at[idx], vmem.at[idx], sems.at[sem])

    def wait(vmem, sem, *idx):
        region = vmem.at[idx] if idx else vmem
        pltpu.make_async_copy(region, region, sems.at[sem]).wait()

    def pair(k):
        return pl.ds(2 * k, 2)

    def ffn_tile(t):
        assert n_fb == 9
        r = (t * 57) >> 9
        return r, t - r * n_fb

    def q_copies(t):
        return [copy(wq_hbm, wq_v, _S_Q, pair(k), pl.ds(t, 1)) for k in range(4)]

    def uk_uv_copies(t):
        return [
            copy(hbm, vmem, sem, pair(k), pl.ds(t, 1))
            for k in range(2)
            for hbm, vmem, sem in ((wuk_hbm, wuk_v, _S_UK), (wuv_hbm, wuv_v, _S_UV))
        ]

    def kv_copies(half):
        return lambda t: [
            copy(kv_hbm, kv_v, _S_KV + half, pair(4 * (t & 1) + k),
                 _aligned(half * half_slab + 8 * (t >> 1), 8, 8))
            for k in range(4)
        ]

    def gate_up_copies(t):
        r, c = ffn_tile(t)
        return [
            copy(hbm, vmem, sem, pair(k), _aligned(8 * r, 8, 8), _aligned(_FB * c, _FB, _FB))
            for k in range(2)
            for hbm, vmem, sem in ((wg_hbm, wg_v, _S_G), (wu_hbm, wu_v, _S_U))
        ]

    def down_copies(t):
        r, c = ffn_tile(t)
        return [
            copy(wd_hbm, wd_v, _S_D, pair(k),
                 _aligned(8 * r + (fr // 2) * j, 8, 8), _aligned(_FB * c, _FB, _FB))
            for j in range(2)
            for k in range(2)
        ]

    wo_ends = [(g * m_dim + c1) // 32 for ((_, _, g, _, c1),) in _WO_REGULAR]

    def o_copies(t):
        sem = _S_O
        for end in wo_ends[:-1]:
            sem = sem + (t >= end if isinstance(t, int) else (t >= end).astype(jnp.int32))
        return [copy(wo_hbm, wo_v, sem, pair(k), _aligned(32 * t, 32, 32)) for k in range(4)]

    def own_head(n_cols):
        shape = (rows, n_cols)
        return _iota(shape, 0) % _HG == _iota(shape, 1) % _HG

    def head_group(w_ref, i, g):
        w = w_ref[i, :, g * _HG:(g + 1) * _HG, :]
        return w.reshape(w.shape[0] * _HG, d_head)

    stage = _Stage(qb, q_copies)
    stage.ticks(1)
    pltpu.make_async_copy(x_hbm, x_v, sems.at[_S_X]).start()
    pltpu.make_async_copy(wr_hbm, wr_v, sems.at[_S_WR]).start()

    def init_step(i, carry):
        shape = (16, e_ref.shape[1])
        e_ref[_aligned(16 * i, 16, 16), :] = jnp.where(
            _iota(shape, 1) // _HG == _iota(shape, 0) + 16 * i, 1.0, 0.0
        ).astype(_BF16)
        xb_ref[i] = jnp.zeros(xb_ref.shape[1:], _BF16)
        return carry

    assert e_ref.shape[0] == 16 * n_qb
    stage.loop(n_qb, 1, init_step, 0)
    stage.idle(_LAG + 1 - stage.issued)

    wait(x_v, _S_X)
    x = x_v[...].astype(_F32)
    mean = jnp.mean(x, axis=-1, keepdims=True)
    xc = x - mean
    var = jnp.mean(xc * xc, axis=-1, keepdims=True)
    xn = xc / jnp.sqrt(var + 1e-5)

    def repeat_rows(v, n_rows, rep):
        row = _iota((n_rows, m_dim), 0) // rep
        out = jnp.zeros((n_rows, m_dim), _F32)
        for b in range(nb):
            out = jnp.where(row == b, v[b:b + 1, :], out)
        return out

    xn_rep = repeat_rows(xn, rows, _HG)
    for i in range(n_qb):
        xb_ref[i, :, 0:qb] = xn_rep[:, i * qb:(i + 1) * qb].astype(_BF16)
    x8 = repeat_rows(x, 8, 1)
    xn8 = repeat_rows(xn, 8, 1)
    stage.ticks(2)

    wait(wr_v, _S_WR)
    w_r = wr_v[...].astype(_F32).reshape(1, m_dim)
    route = _sigmoid(jnp.sum(xn8 * w_r, axis=-1, keepdims=True))
    stage.finish()

    stage = _Stage(cb, uk_uv_copies)
    stage.idle(_LAG)
    wait(wq_v, _S_Q)

    def q_step(i, acc):
        spread = _dot(xb_ref[i], e_ref[:, 0:qb * _HG])
        lhs = jnp.where(own_head(qb * _HG), spread, 0.0).astype(_BF16)
        return tuple(acc[g] + _dot(lhs, head_group(wq_v, i, g)) for g in range(n_groups))

    q = stage.loop(
        n_qb, 6, q_step, tuple(jnp.zeros((rows, d_head), _F32) for _ in range(n_groups))
    )
    q = [(qg * (d_head ** -0.5)).astype(_BF16) for qg in q]
    stage.finish()

    stage = _Stage(kb // 8, kv_copies(0))
    stage.idle(_LAG)
    wait(wuk_v, _S_UK)

    def uk_step(j, carry):
        for g in range(n_groups):
            full = _dot_nt(q[g], head_group(wuk_v, j, g))
            own = jnp.where(own_head(cb * _HG), full, 0.0).astype(_BF16)
            qa_ref[j, g] = _dot_nt(own, e_ref[...]).astype(_BF16)
        return carry

    stage.loop(n_cb, 12, uk_step, 0)
    stage.finish()

    def keys(b, half):
        slabs = pl.ds(b * slabs_per_batch, slabs_per_batch)
        k = kv_v[slabs, _aligned(half * half_slab, half_slab, half_slab), :]
        return k.reshape(slabs_per_batch * half_slab, d_lat)

    def head_rows(b):
        return _aligned(b * _HG, _HG, _HG)

    def score_step(half, b, carry):
        qa = jnp.concatenate(
            [
                jnp.concatenate([qa_ref[j, g, head_rows(b), :] for j in range(n_cb)], axis=1)
                for g in range(n_groups)
            ],
            axis=0,
        )
        s = _dot_nt(qa, keys(b, half))
        s_ref[2 * b + half] = s
        m = s[:, 0:128] if half == 0 else jnp.maximum(m_ref[b], s[:, 0:128])
        for t in range(1, s.shape[1] // 128):
            m = jnp.maximum(m, s[:, t * 128:(t + 1) * 128])
        m_ref[b] = m
        return carry

    stage = _Stage(kb // 8, kv_copies(1))
    stage.idle(_LAG)
    wait(kv_v, _S_KV, pl.ds(0, n_slabs), pl.ds(0, half_slab))
    stage.loop(nb, 10, functools.partial(score_step, 0), 0)
    stage.finish()

    stage = _Stage((fr // 8) * n_fb, gate_up_copies)
    stage.idle(_LAG)
    wait(kv_v, _S_KV + 1, pl.ds(0, n_slabs), pl.ds(half_slab, half_slab))
    stage.loop(nb, 10, functools.partial(score_step, 1), 0)

    def value_step(i, carry):
        b, half = i >> 1, i & 1
        l, acc = (jnp.where(half == 1, v, 0.0) for v in carry)
        p = jnp.exp(s_ref[i] - jnp.max(m_ref[b], axis=-1, keepdims=True))
        for t in range(p.shape[1] // 128):
            l = l + p[:, t * 128:(t + 1) * 128]
        acc = acc + _dot(p.astype(_BF16), keys(b, half))
        cc = (acc / jnp.sum(l, axis=-1, keepdims=True)).astype(_BF16)
        for g in range(n_groups):
            for j in range(n_cb):
                cc_ref[j, g, head_rows(b), :] = cc[g * _HG:(g + 1) * _HG, j * cb:(j + 1) * cb]
        return l, acc

    stage.loop(
        2 * nb, 6, value_step,
        (jnp.zeros((n_heads, 128), _F32), jnp.zeros((n_heads, d_lat), _F32)),
    )
    wait(wuv_v, _S_UV)

    def uv_step(j, acc):
        out = []
        for g in range(n_groups):
            spread = _dot(cc_ref[j, g], e_ref[...])
            lhs = jnp.where(own_head(cb * _HG), spread, 0.0).astype(_BF16)
            out.append(acc[g] + _dot(lhs, head_group(wuv_v, j, g)))
        return tuple(out)

    ctx = stage.loop(
        n_cb, 12, uv_step, tuple(jnp.zeros((rows, d_head), _F32) for _ in range(n_groups))
    )
    dst, src = _iota((8 * _HG, rows), 0), _iota((8 * _HG, rows), 1)
    regroup = jnp.where(
        (dst // 8 == src % _HG) & (dst % 8 == src // _HG), 1.0, 0.0
    ).astype(_BF16)
    for g in range(n_groups):
        ctx_ref[g * 8 * _HG:(g + 1) * 8 * _HG, :] = _dot(regroup, ctx[g].astype(_BF16))
    stage.finish()

    stage = _Stage((fr // 16) * n_fb, down_copies)
    stage.idle(_LAG)
    wait(wg_v, _S_G)
    wait(wu_v, _S_U)
    xn8_bf16 = xn8.astype(_BF16)

    def ffn_cols(w_ref, start, size):
        return w_ref[:, :, _aligned(start, size, _FB)].reshape(m_dim, size)

    def up_step(i, carry):
        gate = _dot(xn8_bf16, ffn_cols(wg_v, i * _FB, _FB))
        h_ref[i] = gate * _sigmoid(gate) * _dot(xn8_bf16, ffn_cols(wu_v, i * _FB, _FB))
        return carry

    stage.loop(n_fb, 5, up_step, 0)
    stage.finish()

    stage = _Stage(wo_ends[-1], o_copies)
    stage.idle(_LAG - 3)
    wait(wd_v, _S_D)

    def down_step(i, acc):
        h = jnp.concatenate([h_ref[3 * i + k] for k in range(3)], axis=1)
        return acc + _dot_nt(h.astype(_BF16), ffn_cols(wd_v, i * 3 * _FB, 3 * _FB))

    y = stage.loop(n_fb // 3, 8, down_step, jnp.zeros((8, m_dim), _F32))
    z = xn8 + (xn8 * 0.0 + y * route)
    gate = z * _sigmoid(z)

    pending = [c for t in range(stage.issued, stage.n_ticks) for c in o_copies(t)]
    piece_ends = [4 * (end - stage.issued) for end in wo_ends]
    sem = _S_O + len(_WO_REGULAR)
    for piece in _WO_FINAL:
        for k0, nk, g, c0, c1 in piece:
            dk, dc = (2, 32) if nk % 2 == 0 else (1, 64)
            pending += [
                copy(wo_hbm, wo_v, sem, pl.ds(k, dk), pl.ds(g * m_dim + c, dc))
                for c in range(c0, c1, dc)
                for k in range(k0, k0 + nk, dk)
            ]
            sem += 1
        piece_ends.append(len(pending))
    n_started = [0]

    def start_until(n):
        for i in range(n_started[0], min(n, len(pending))):
            in_order = i >= len(pending) - _WO_IN_ORDER
            pending[i].start(priority=1 if in_order else _PRIORITY[i % 4])
            n_started[0] = i + 1

    pieces = _WO_REGULAR + _WO_FINAL
    blocks = [block for piece in pieces for block in piece]
    col_tiles = [(c, min(c + 128, m_dim)) for c in range(0, m_dim, 128)]
    s = [jnp.zeros((8, c1 - c0), _F32) for c0, c1 in col_tiles]
    heads_per_slab = n_heads // wo_v.shape[0]
    n_done = 0
    for piece, end in zip(pieces, piece_ends, strict=True):
        start_until(end + 4 * (_LAG - 3))
        for i, (k0, nk, g, c0, c1) in enumerate(piece):
            wait(wo_v, _S_O + n_done + i, pl.ds(k0, nk), pl.ds(g * m_dim + c0, c1 - c0))
        for k0, nk, g, c0, c1 in piece:
            n_done += 1
            part = None
            for k in range(k0, k0 + nk):
                head = k * heads_per_slab + g
                term = _dot_nt(
                    ctx_ref[8 * head:8 * head + 8, :].astype(_BF16),
                    wo_v[k, g * m_dim + c0:g * m_dim + c1, :],
                )
                part = term if part is None else part + term
                start_until(n_started[0] + 3)
            for n, (t0, t1) in enumerate(col_tiles):
                if c0 <= t0 and t1 <= c1:
                    s[n] = s[n] + part[:, t0 - c0:t1 - c0]
                    if not any(b0 <= t0 and t1 <= b1 for *_, b0, b1 in blocks[n_done:]):
                        out = x8[:, t0:t1] + s[n] * gate[:, t0:t1]
                        out_v[:, t0:t1] = out.astype(out_v.dtype)[0:nb]
    assert n_started[0] == len(pending)

    write_back = pltpu.make_async_copy(out_v, o_hbm, sems.at[_S_X])
    write_back.start()
    write_back.wait()


@jax.jit
def pallas_recurrent_scan__compressed_kv_cla__moe_arch_mod__decode_kernel(
    A_x: jax.Array,
    A_c_kv: jax.Array,
    A_w_q: jax.Array,
    A_w_uk: jax.Array,
    A_w_uv: jax.Array,
    A_w_o: jax.Array,
    B_x: jax.Array,
    B_w_r: jax.Array,
    B_w_gate: jax.Array,
    B_w_up: jax.Array,
    B_w_down: jax.Array,
):
    del B_x
    nb, sq, m_dim = A_x.shape
    _, n_keys, d_lat = A_c_kv.shape
    _, n_heads, d_head = A_w_q.shape
    d_ff = B_w_gate.shape[1]
    assert (nb, sq, m_dim, n_keys, d_lat) == (4, 1, 576, 4096, 512)
    assert (n_heads, d_head, d_ff) == (32, 128, 4608)
    n_groups = n_heads // _HG
    rows = nb * _HG

    operands = (
        A_x.reshape(nb, m_dim),
        B_w_r,
        A_w_q.reshape(8, m_dim // 8, n_heads, d_head),
        A_w_uk.reshape(4, d_lat // 4, n_heads, d_head),
        A_w_uv.reshape(4, d_lat // 4, n_heads, d_head),
        A_c_kv.reshape(16, nb * n_keys // 16, d_lat),
        B_w_gate.reshape(4, m_dim // 4, d_ff),
        B_w_up.reshape(4, m_dim // 4, d_ff),
        B_w_down.T.reshape(4, m_dim // 4, d_ff),
        jnp.transpose(A_w_o, (0, 2, 1)).reshape(8, n_heads * m_dim // 8, d_head),
    )
    scratch = [pltpu.VMEM(a.shape, a.dtype) for a in operands] + [
        pltpu.VMEM((128, 128 * _HG), _BF16),
        pltpu.VMEM((8, rows, 128), _BF16),
        pltpu.VMEM((4, n_groups, rows, d_lat // 4), _BF16),
        pltpu.VMEM((2 * nb, n_heads, n_keys // 2), _F32),
        pltpu.VMEM((nb, n_heads, 128), _F32),
        pltpu.VMEM((4, n_groups, rows, d_lat // 4), _BF16),
        pltpu.VMEM((8 * n_heads, d_head), _F32),
        pltpu.VMEM((d_ff // _FB, 8, _FB), _F32),
        pltpu.VMEM((nb, m_dim), A_x.dtype),
        pltpu.SemaphoreType.DMA((_N_SEMS,)),
    ]
    out = pl.pallas_call(
        _kernel,
        out_shape=jax.ShapeDtypeStruct((nb, m_dim), A_x.dtype),
        in_specs=[pl.BlockSpec(memory_space=pltpu.HBM)] * len(operands),
        out_specs=pl.BlockSpec(memory_space=pltpu.HBM),
        scratch_shapes=scratch,
        compiler_params=pltpu.CompilerParams(
            vmem_limit_bytes=100 * 2**20,
            disable_semaphore_checks=True,
            disable_bounds_checks=True,
        ),
    )(*operands)
    return out.reshape(nb, sq, m_dim)
```
